```python
import jax
import jax.numpy as jnp

def _softmax(x, axis=-1):
    return jax.nn.softmax(x, axis=axis)
def _gelu(x):
    return jax.nn.gelu(x, approximate=True)
def _silu(x):
    return jax.nn.silu(x)
def _sigmoid(x):
    return jax.nn.sigmoid(x)
def _layernorm(x, axis=-1, eps=1e-5):
    m = jnp.mean(x, axis=axis, keepdims=True)
    v = jnp.var(x, axis=axis, keepdims=True)
    return (x - m) / jnp.sqrt(v + eps)
def _scatter_add(tgt, idx, src, axis=0):
    return tgt.at[idx].add(src)
def _segment_sum(src, seg, n):
    return jax.ops.segment_sum(src, seg, n)
class _Rng:
    def __init__(self, key):
        self._k = key
    def _next(self):
        self._k, sub = jax.random.split(self._k)
        return sub
    def normal(self, shape):
        return jax.random.normal(self._next(), shape, dtype=jnp.bfloat16)
    def randint(self, lo, hi, shape):
        return jax.random.randint(self._next(), shape, lo, hi, dtype=jnp.int32)
    def uniform(self, shape, lo=0.0, hi=1.0):
        return jax.random.uniform(self._next(), shape, jnp.bfloat16, lo, hi)
    def permutation(self, n):
        return jax.random.permutation(self._next(), n)


kernel_name = 'recurrent_scan__sliding_block_cached__moe_arch_mod__prompt'

def setup_inputs():
    _rng = _Rng(jax.random.key(int.from_bytes(__import__("os").urandom(4), "little")))
    _w = (lambda a: (lambda t: t.astype(jnp.bfloat16) if jnp.issubdtype(t.dtype, jnp.floating) else t)(jnp.asarray(a)))
    def _A_setup():
        B, Sq, D = 1, 2048, 640
        Hq, Hkv, Sk, Dh = 32, 32, 2048, 192
        assert Hq % Hkv == 0, (Hq, Hkv)
        return {
            "x": _w((lambda *s: _rng.normal(s) * 0.05)(B, Sq, D)),
            "k_cache": _w((lambda *s: _rng.normal(s) * 0.05)(B, Hkv, Sk, Dh)),
            "v_cache": _w((lambda *s: _rng.normal(s) * 0.05)(B, Hkv, Sk, Dh)),
            "wq": _w((lambda *s: _rng.normal(s) * 0.05)(D, Hq * Dh) * (D ** -0.5)),
            "wo": _w((lambda *s: _rng.normal(s) * 0.05)(Hq * Dh, D) * ((Hq * Dh) ** -0.5)),
        }
    _A_in = _A_setup()

    def _B_setup():
        B, S, D, F, C = 1, 2048, 640, 1536, 2
        return {
            "x": _w((lambda *s: _rng.normal(s) * 0.05)(B, S, D)),
            "w_r": _w((lambda *s: _rng.normal(s) * 0.05)(D)),
            "w_gate": _w((lambda *s: _rng.normal(s) * 0.05)(D, F)),
            "w_up": _w((lambda *s: _rng.normal(s) * 0.05)(D, F)),
            "w_down": _w((lambda *s: _rng.normal(s) * 0.05)(F, D)),
        }
    _B_in = _B_setup()

    return {
        "A_x": _A_in["x"],
        "A_k_cache": _A_in["k_cache"],
        "A_v_cache": _A_in["v_cache"],
        "A_wq": _A_in["wq"],
        "A_wo": _A_in["wo"],
        "B_x": _B_in["x"],
        "B_w_r": _B_in["w_r"],
        "B_w_gate": _B_in["w_gate"],
        "B_w_up": _B_in["w_up"],
        "B_w_down": _B_in["w_down"],
    }

def reference(A_x, A_k_cache, A_v_cache, A_wq, A_wo, B_x, B_w_r, B_w_gate, B_w_up, B_w_down):
    def _A_ref(x, k_cache, v_cache, wq, wo):
        B, Sq, D = x.shape
        Hq, Dh = 32, 192
        Hkv, Sk = k_cache.shape[1], k_cache.shape[2]
        W = min(4096, max(256, Sk // 4))
        rep = Hq // Hkv
        q = (lambda x, *d: x.transpose(*d))((x @ wq).reshape(B, Sq, Hq, Dh), 0, 2, 1, 3)
        k = jnp.repeat(k_cache[:, :, Sk - W:, :], rep, axis=1)
        v = jnp.repeat(v_cache[:, :, Sk - W:, :], rep, axis=1)
        scores = jnp.einsum("bhqd,bhkd->bhqk", q, k) * (Dh ** -0.5)
        p = _softmax(scores, axis=-1)
        o = jnp.einsum("bhqk,bhkd->bhqd", p, v)
        return (lambda x, *d: x.transpose(*d))(o, 0, 2, 1, 3).reshape(B, Sq, Hq * Dh) @ wo

    def _B_ref(x, w_r, w_gate, w_up, w_down):
        B, S, D = x.shape
        C = 2
        r = x @ w_r
        idx = jnp.argsort(-r, axis=-1)[:, :C]
        idx_e = jnp.repeat(idx.reshape(B, C, 1), D, axis=2)
        x_sel = jnp.take_along_axis(x, idx_e, axis=1)
        g = _silu(x_sel @ w_gate)
        u = x_sel @ w_up
        y = (g * u) @ w_down
        r_sel = _sigmoid(jnp.take_along_axis(r, idx, axis=1))
        y = y * r_sel.reshape(B, C, 1)
        b_off = (jnp.arange(B) * S).reshape(B, 1)
        flat_idx = (idx + b_off).reshape(B * C)
        zero = (x * 0.0).reshape(B * S, D)
        upd = _scatter_add(zero, flat_idx, y.reshape(B * C, D), axis=0)
        return x + upd.reshape(B, S, D)

    x = A_x
    xn = _layernorm(x, axis=-1)
    s = _A_ref(xn, A_k_cache, A_v_cache, A_wq, A_wo)
    g = _silu(_B_ref(xn, B_w_r, B_w_gate, B_w_up, B_w_down))
    return x + s * g
```

```python
import functools
import jax
import jax.numpy as jnp
from jax import lax
import jax.experimental.pallas as pl
import jax.experimental.pallas.tpu as pltpu

S, D, H, DH, SK, W, F = 2048, 640, 32, 192, 2048, 512, 1536
NP = H // 2
LOG2E = 1.4426950408889634
NN = (((1,), (0,)), ((), ()))
NT = (((1,), (1,)), ((), ()))
TN = (((0,), (0,)), ((), ()))
f32 = jnp.float32
bf16 = jnp.bfloat16


def make(bm=512, vmem=100, mode="N", hbm=True, unroll=1):
    nsub = S // bm

    def kernel(x_ref, k_ref, v_ref, wq_ref, wo_ref, wr_ref, wg_ref, wu_ref, wd_ref, o_ref,
               xn_ref, acc_ref, upd_ref, idx_ref):
        p = pl.program_id(0)

        @pl.when(p == 0)
        def _prologue():
            def ln(i, carry):
                r0 = pl.multiple_of(i * bm, bm)
                x = x_ref[pl.ds(r0, bm), :].astype(f32)
                m = jnp.mean(x, axis=-1, keepdims=True)
                d = x - m
                v = jnp.mean(d * d, axis=-1, keepdims=True)
                xn = (d / jnp.sqrt(v + 1e-5)).astype(bf16)
                xn_ref[pl.ds(r0, bm), :] = xn
                return carry
            lax.fori_loop(0, nsub, ln, 0)
            wr = wr_ref[...].astype(f32)
            r = jnp.sum(xn_ref[...].astype(f32) * wr, axis=-1, keepdims=True)
            r = r.astype(bf16).astype(f32)
            ii = lax.broadcasted_iota(jnp.int32, (S, 1), 0)
            m1 = jnp.max(r, axis=0, keepdims=True)
            i1 = jnp.min(jnp.where(r == m1, ii, S), axis=0, keepdims=True)
            r2 = jnp.where(ii == i1, -jnp.inf, r)
            m2 = jnp.max(r2, axis=0, keepdims=True)
            i2 = jnp.min(jnp.where(r2 == m2, ii, S), axis=0, keepdims=True)
            idx_ref[0] = i1[0, 0]
            idx_ref[1] = i2[0, 0]
            xnf = xn_ref[...].astype(f32)
            xs1 = jnp.sum(jnp.where(ii == i1, xnf, 0.0), axis=0, keepdims=True)
            xs2 = jnp.sum(jnp.where(ii == i2, xnf, 0.0), axis=0, keepdims=True)
            row = lax.broadcasted_iota(jnp.int32, (8, D), 0)
            xs = jnp.where(row == 0, xs1, jnp.where(row == 1, xs2, 0.0)).astype(bf16)
            g = jnp.dot(xs, wg_ref[...], preferred_element_type=f32)
            u = jnp.dot(xs, wu_ref[...], preferred_element_type=f32)
            hmid = (g * jax.nn.sigmoid(g) * u).astype(bf16)
            y = jnp.dot(hmid, wd_ref[...], preferred_element_type=f32)
            rs = jnp.where(row[:, :1] == 0, m1, m2)
            upd_ref[...] = y * jax.nn.sigmoid(rs)
            acc_ref[...] = jnp.zeros_like(acc_ref)

        z = jnp.zeros((64, W), bf16)
        k0p = jnp.concatenate([k_ref[0], z], axis=0)
        k1p = jnp.concatenate([z, k_ref[1]], axis=0)
        if mode == "N":
            v0p = jnp.concatenate([v_ref[0], z], axis=0)
            v1p = jnp.concatenate([z, v_ref[1]], axis=0)
        else:
            v0p = v_ref[0]
            v1p = v_ref[1]
        if mode == "M2":
            woT = wo_ref[...].T
        c = (DH ** -0.5) * LOG2E

        def body(i, carry):
            r0 = pl.multiple_of(i * bm, bm)
            xn = xn_ref[pl.ds(r0, bm), :]
            q = (jnp.dot(xn, wq_ref[...], preferred_element_type=f32) * c).astype(bf16)
            outs = []
            for (qq, kk, vv) in ((q[:, 0:256], k0p, v0p), (q[:, 128:384], k1p, v1p)):
                s = jnp.dot(qq, kk, preferred_element_type=f32)
                m = jnp.max(s, axis=-1, keepdims=True)
                e = jnp.exp2(s - m)
                l = jnp.sum(e, axis=-1, keepdims=True)
                if mode == "N":
                    o = lax.dot_general(e.astype(bf16), vv, NT, preferred_element_type=f32)
                    outs.append(o * (1.0 / l))
                else:
                    pn = (e * (1.0 / l)).astype(bf16)
                    oT = lax.dot_general(vv, pn, NT, preferred_element_type=f32)
                    outs.append(oT.astype(bf16))
            o0, o1 = outs
            if mode == "N":
                o = jnp.concatenate([o0[:, :128], o0[:, 128:] + o1[:, :128], o1[:, 128:]], axis=1).astype(bf16)
                acc_ref[pl.ds(r0, bm), :] += jnp.dot(o, wo_ref[...], preferred_element_type=f32)
            elif mode == "M1":
                oT = jnp.concatenate([o0, o1], axis=0)
                acc_ref[pl.ds(r0, bm), :] += lax.dot_general(oT, wo_ref[...], TN, preferred_element_type=f32)
            elif mode == "M2":
                oT = jnp.concatenate([o0, o1], axis=0)
                acc_ref[:, pl.ds(r0, bm)] += jnp.dot(woT, oT, preferred_element_type=f32)
            return carry
        lax.fori_loop(0, nsub, body, 0, unroll=unroll)

        @pl.when(p == NP - 1)
        def _epilogue():
            def fin(i, carry):
                r0 = pl.multiple_of(i * bm, bm)
                xn = xn_ref[pl.ds(r0, bm), :].astype(f32)
                ii = r0 + lax.broadcasted_iota(jnp.int32, (bm, 1), 0)
                b = xn + jnp.where(ii == idx_ref[0], upd_ref[0:1, :], 0.0) + jnp.where(ii == idx_ref[1], upd_ref[1:2, :], 0.0)
                g = b * jax.nn.sigmoid(b)
                x = x_ref[pl.ds(r0, bm), :].astype(f32)
                if mode == "M2":
                    a = acc_ref[:, pl.ds(r0, bm)].T
                else:
                    a = acc_ref[pl.ds(r0, bm), :]
                o_ref[pl.ds(r0, bm), :] = (x + a * g).astype(o_ref.dtype)
                return carry
            lax.fori_loop(0, nsub, fin, 0)

    def fn(A_x, A_k_cache, A_v_cache, A_wq, A_wo, B_x, B_w_r, B_w_gate, B_w_up, B_w_down):
        x2 = A_x.reshape(S, D)
        kT = jnp.swapaxes(A_k_cache, 2, 3)
        vT = jnp.swapaxes(A_v_cache, 2, 3)
        full = lambda shape: pl.BlockSpec(shape, lambda p: (0,) * len(shape))
        args = [x2, kT, vT, A_wq, A_wo, B_w_r.reshape(1, D), B_w_gate, B_w_up, B_w_down]
        if hbm:
            args = [pltpu.with_memory_space_constraint(a, pltpu.HBM) for a in args]
        out = pl.pallas_call(
            kernel,
            grid=(NP,),
            in_specs=[
                full((S, D)),
                pl.BlockSpec((None, 2, DH, W), lambda p: (0, p, 0, SK // W - 1)),
                pl.BlockSpec((None, 2, DH, W), lambda p: (0, p, 0, SK // W - 1)),
                pl.BlockSpec((D, 2 * DH), lambda p: (0, p)),
                pl.BlockSpec((2 * DH, D), lambda p: (p, 0)),
                full((1, D)),
                full((D, F)), full((D, F)), full((F, D)),
            ],
            out_specs=full((S, D)),
            out_shape=jax.ShapeDtypeStruct((S, D), jnp.bfloat16),
            scratch_shapes=[
                pltpu.VMEM((S, D), jnp.bfloat16),
                pltpu.VMEM((D, S) if mode == "M2" else (S, D), jnp.float32),
                pltpu.VMEM((8, D), jnp.float32),
                pltpu.SMEM((2,), jnp.int32),
            ],
            compiler_params=pltpu.CompilerParams(
                dimension_semantics=("arbitrary",), vmem_limit_bytes=vmem * 1024 * 1024),
        )(*args)
        return out.reshape(1, S, D)
    return fn


_fn = make(bm=512, unroll=2)


@jax.jit
def pallas_recurrent_scan__sliding_block_cached__moe_arch_mod__prompt_kernel(A_x, A_k_cache, A_v_cache, A_wq, A_wo, B_x, B_w_r, B_w_gate, B_w_up, B_w_down):
    return _fn(A_x, A_k_cache, A_v_cache, A_wq, A_wo, B_x, B_w_r, B_w_gate, B_w_up, B_w_down)
```

```python
import functools
import jax
import jax.numpy as jnp
from jax import lax
import jax.experimental.pallas as pl
import jax.experimental.pallas.tpu as pltpu

S, D, H, DH, SK, W, F = 2048, 640, 32, 192, 2048, 512, 1536
LOG2E = 1.4426950408889634
NN = (((1,), (0,)), ((), ()))
NT = (((1,), (1,)), ((), ()))
TN = (((0,), (0,)), ((), ()))
f32 = jnp.float32
bf16 = jnp.bfloat16


def make(bm=512, vmem=100, NP=H // 2, xc=256, unroll=4, oc=256, rstep=2):
    nsub = S // bm
    nxc = S // xc
    noc = S // oc
    rstep = min(rstep, NP - 1)

    def kernel(x_hbm, k_ref, v_ref, wq_ref, wo_ref, wr_ref, wg_hbm, wu_hbm, wd_hbm, o_hbm,
               xbuf, xn_ref, acc_ref, obuf, r_ref, wg_ref, wu_ref, wd_ref, upd_ref, idx_ref,
               xsem, wsem, osem):
        p = pl.program_id(0)

        def x_copy(i):
            r0 = pl.multiple_of(i * xc, xc)
            return pltpu.make_async_copy(x_hbm.at[pl.ds(r0, xc), :], xbuf.at[pl.ds(r0, xc), :], xsem.at[i])

        def o_copy(i):
            r0 = pl.multiple_of(i * oc, oc)
            return pltpu.make_async_copy(obuf.at[pl.ds(r0, oc), :], o_hbm.at[pl.ds(r0, oc), :], osem.at[i])

        def w_copies():
            return [pltpu.make_async_copy(wg_hbm, wg_ref, wsem.at[0]),
                    pltpu.make_async_copy(wu_hbm, wu_ref, wsem.at[1]),
                    pltpu.make_async_copy(wd_hbm, wd_ref, wsem.at[2])]

        @pl.when(p == 0)
        def _prologue():
            for i in range(nxc):
                x_copy(i).start()
            for cp in w_copies():
                cp.start()

            def ln(i, carry):
                x_copy(i).wait()
                sl = pl.ds(pl.multiple_of(i * xc, xc), xc)
                x = xbuf[sl, :].astype(f32)
                m = jnp.mean(x, axis=-1, keepdims=True)
                d = x - m
                v = jnp.mean(d * d, axis=-1, keepdims=True)
                xn = (d / jnp.sqrt(v + 1e-5)).astype(bf16)
                xn_ref[sl, :] = xn
                wr = wr_ref[...].astype(f32)
                r_ref[sl, :] = jnp.sum(xn.astype(f32) * wr, axis=-1, keepdims=True)
                acc_ref[sl, :] = jnp.zeros((xc, D), f32)
                return carry
            lax.fori_loop(0, nxc, ln, 0)

        @pl.when(p == rstep)
        def _router():
            r = r_ref[...].astype(bf16).astype(f32)
            ii = lax.broadcasted_iota(jnp.int32, (S, 1), 0)
            m1 = jnp.max(r, axis=0, keepdims=True)
            i1 = jnp.min(jnp.where(r == m1, ii, S - 1), axis=0, keepdims=True)
            r2 = jnp.where(ii == i1, -jnp.inf, r)
            m2 = jnp.max(r2, axis=0, keepdims=True)
            i2 = jnp.min(jnp.where(r2 == m2, ii, S - 1), axis=0, keepdims=True)
            s1 = i1[0, 0]
            s2 = i2[0, 0]
            idx_ref[0] = s1
            idx_ref[1] = s2
            b1 = pl.multiple_of((s1 // 16) * 16, 16)
            b2 = pl.multiple_of((s2 // 16) * 16, 16)
            row = lax.broadcasted_iota(jnp.int32, (16, D), 0)
            x1 = jnp.sum(jnp.where(row == s1 - b1, xn_ref[pl.ds(b1, 16), :].astype(f32), 0.0), axis=0, keepdims=True)
            x2 = jnp.sum(jnp.where(row == s2 - b2, xn_ref[pl.ds(b2, 16), :].astype(f32), 0.0), axis=0, keepdims=True)
            xs = jnp.where(row == 0, x1, jnp.where(row == 1, x2, 0.0)).astype(bf16)
            for c in w_copies():
                c.wait()
            g = jnp.dot(xs, wg_ref[...], preferred_element_type=f32)
            u = jnp.dot(xs, wu_ref[...], preferred_element_type=f32)
            hmid = (g * jax.nn.sigmoid(g) * u).astype(bf16)
            y = jnp.dot(hmid, wd_ref[...], preferred_element_type=f32)
            rs = jnp.where(row[:, :1] == 0, m1, m2)
            upd_ref[...] = y * jax.nn.sigmoid(rs)

        c = (DH ** -0.5) * LOG2E
        z = jnp.zeros((64, W), bf16)
        k0p = jnp.concatenate([k_ref[0], z], axis=0).T
        k1p = jnp.concatenate([z, k_ref[1]], axis=0).T

        def body(i, carry):
            sl = pl.ds(pl.multiple_of(i * bm, bm), bm)
            xn = xn_ref[sl, :]
            q = (jnp.dot(xn, wq_ref[...], preferred_element_type=f32) * c).astype(bf16)
            outs = []
            for (qq, kk, h) in ((q[:, 0:256], k0p, 0), (q[:, 128:384], k1p, 1)):
                sT = lax.dot_general(kk, qq, NT, preferred_element_type=f32)
                m = jnp.max(sT, axis=0, keepdims=True)
                e = jnp.exp2(sT - m)
                l = jnp.sum(e, axis=0, keepdims=True)
                oT = jnp.dot(v_ref[h], e.astype(bf16), preferred_element_type=f32)
                outs.append((oT * (1.0 / l)).astype(bf16))
            oT = jnp.concatenate(outs, axis=0)
            acc_ref[sl, :] += lax.dot_general(oT, wo_ref[...], TN, preferred_element_type=f32)
            return carry
        lax.fori_loop(0, nsub, body, 0, unroll=unroll)

        @pl.when(p == NP - 1)
        def _epilogue():
            def fin(i, carry):
                r0 = pl.multiple_of(i * oc, oc)
                sl = pl.ds(r0, oc)
                ii = r0 + lax.broadcasted_iota(jnp.int32, (oc, 1), 0)
                b = xn_ref[sl, :].astype(f32) + jnp.where(ii == idx_ref[0], upd_ref[0:1, :], 0.0) \
                    + jnp.where(ii == idx_ref[1], upd_ref[1:2, :], 0.0)
                g = b * jax.nn.sigmoid(b)
                obuf[sl, :] = (xbuf[sl, :].astype(f32) + acc_ref[sl, :] * g).astype(bf16)
                o_copy(i).start()
                return carry
            lax.fori_loop(0, noc, fin, 0)
            for i in range(noc):
                o_copy(i).wait()

    def fn(A_x, A_k_cache, A_v_cache, A_wq, A_wo, B_x, B_w_r, B_w_gate, B_w_up, B_w_down):
        x2 = A_x.reshape(S, D)
        kT = jnp.swapaxes(A_k_cache, 2, 3)
        vT = jnp.swapaxes(A_v_cache, 2, 3)
        anyspec = pl.BlockSpec(memory_space=pltpu.HBM)
        args = [x2, kT, vT, A_wq, A_wo, B_w_r.reshape(1, D), B_w_gate, B_w_up, B_w_down]
        args = [pltpu.with_memory_space_constraint(a, pltpu.HBM) for a in args]
        out = pl.pallas_call(
            kernel,
            grid=(NP,),
            in_specs=[
                anyspec,
                pl.BlockSpec((None, 2, DH, W), lambda p: (0, p, 0, SK // W - 1)),
                pl.BlockSpec((None, 2, DH, W), lambda p: (0, p, 0, SK // W - 1)),
                pl.BlockSpec((D, 2 * DH), lambda p: (0, p)),
                pl.BlockSpec((2 * DH, D), lambda p: (p, 0)),
                pl.BlockSpec((1, D), lambda p: (0, 0)),
                anyspec, anyspec, anyspec,
            ],
            out_specs=anyspec,
            out_shape=jax.ShapeDtypeStruct((S, D), jnp.bfloat16),
            scratch_shapes=[
                pltpu.VMEM((S, D), bf16),
                pltpu.VMEM((S, D), bf16),
                pltpu.VMEM((S, D), f32),
                pltpu.VMEM((S, D), bf16),
                pltpu.VMEM((S, 1), f32),
                pltpu.VMEM((D, F), bf16), pltpu.VMEM((D, F), bf16), pltpu.VMEM((F, D), bf16),
                pltpu.VMEM((16, D), f32),
                pltpu.SMEM((2,), jnp.int32),
                pltpu.SemaphoreType.DMA((nxc,)),
                pltpu.SemaphoreType.DMA((3,)),
                pltpu.SemaphoreType.DMA((noc,)),
            ],
            compiler_params=pltpu.CompilerParams(
                dimension_semantics=("arbitrary",), vmem_limit_bytes=vmem * 1024 * 1024),
        )(*args)
        return out.reshape(1, S, D)
    return fn


_fn = make(bm=1024, unroll=2)


@jax.jit
def pallas_recurrent_scan__sliding_block_cached__moe_arch_mod__prompt_kernel(A_x, A_k_cache, A_v_cache, A_wq, A_wo, B_x, B_w_r, B_w_gate, B_w_up, B_w_down):
    return _fn(A_x, A_k_cache, A_v_cache, A_wq, A_wo, B_x, B_w_r, B_w_gate, B_w_up, B_w_down)
```

```python
import functools
import jax
import jax.numpy as jnp
from jax import lax
import jax.experimental.pallas as pl
import jax.experimental.pallas.tpu as pltpu

S, D, H, DH, SK, W, F = 2048, 640, 32, 192, 2048, 512, 1536
LOG2E = 1.4426950408889634
NN = (((1,), (0,)), ((), ()))
NT = (((1,), (1,)), ((), ()))
TN = (((0,), (0,)), ((), ()))
f32 = jnp.float32
bf16 = jnp.bfloat16


def make(bm=1024, vmem=110, NP=H // 2, xc=256, oc=256, rstep=2, flags=None, scopes=False):
    nsub = S // bm
    nxc = S // xc
    noc = S // oc
    rstep = min(rstep, NP - 1)
    scope = jax.named_scope if scopes else (lambda name: (lambda f: f))

    def kernel(x_hbm, k_hbm, v_hbm, wq_hbm, wo_hbm, wr_ref, wg_hbm, wu_hbm, wd_hbm, o_hbm,
               xbuf, xn_ref, acc_ref, obuf, r_ref, wg_ref, wu_ref, wd_ref, upd_ref, idx_ref,
               wq_s, k_s, v_s, wo_s, xsem, wsem, osem, psem):

        def x_copy(i):
            r0 = pl.multiple_of(i * xc, xc)
            return pltpu.make_async_copy(x_hbm.at[pl.ds(r0, xc), :], xbuf.at[pl.ds(r0, xc), :], xsem.at[i])

        def o_copy(i):
            r0 = pl.multiple_of(i * oc, oc)
            return pltpu.make_async_copy(obuf.at[pl.ds(r0, oc), :], o_hbm.at[pl.ds(r0, oc), :], osem.at[i])

        def w_copies():
            return [pltpu.make_async_copy(wg_hbm, wg_ref, wsem.at[0]),
                    pltpu.make_async_copy(wu_hbm, wu_ref, wsem.at[1]),
                    pltpu.make_async_copy(wd_hbm, wd_ref, wsem.at[2])]

        def pair_copies(p):
            slot = p % 2
            c0 = pl.multiple_of(p * 384, 128)
            return [
                pltpu.make_async_copy(wq_hbm.at[:, pl.ds(c0, 384)], wq_s.at[slot], psem.at[0, slot]),
                pltpu.make_async_copy(k_hbm.at[0, pl.ds(2 * p, 2), :, pl.ds(SK - W, W)], k_s.at[slot], psem.at[1, slot]),
                pltpu.make_async_copy(v_hbm.at[0, pl.ds(2 * p, 2), :, pl.ds(SK - W, W)], v_s.at[slot], psem.at[2, slot]),
                pltpu.make_async_copy(wo_hbm.at[pl.ds(c0, 384), :], wo_s.at[slot], psem.at[3, slot]),
            ]

        x_copy(0).start()
        x_copy(1).start()
        for cp in pair_copies(0):
            cp.start()
        for i in range(2, nxc):
            x_copy(i).start()

        wr8 = jnp.broadcast_to(wr_ref[...], (8, D))

        @scope("ln")
        def ln_all():
            def ln(i, carry):
                x_copy(i).wait()
                r0 = pl.multiple_of(i * xc, xc)
                sl = pl.ds(r0, xc)
                x = xbuf[sl, :].astype(f32)
                m = jnp.mean(x, axis=-1, keepdims=True)
                d = x - m
                v = jnp.mean(d * d, axis=-1, keepdims=True)
                xn = (d * lax.rsqrt(v + 1e-5)).astype(bf16)
                xn_ref[sl, :] = xn
                r_ref[:, sl] = lax.dot_general(wr8, xn, NT, preferred_element_type=f32)
                acc_ref[sl, :] = jnp.zeros((xc, D), f32)
                return carry
            lax.fori_loop(0, nxc, ln, 0)
        ln_all()

        @scope("router")
        def router():
            r = r_ref[...].astype(bf16).astype(f32)
            ii = lax.broadcasted_iota(jnp.int32, (8, S), 1)
            m1 = jnp.max(r, axis=1, keepdims=True)
            i1 = jnp.min(jnp.where(r == m1, ii, S - 1), axis=1, keepdims=True)
            r2 = jnp.where(ii == i1, -jnp.inf, r)
            m2 = jnp.max(r2, axis=1, keepdims=True)
            i2 = jnp.min(jnp.where(r2 == m2, ii, S - 1), axis=1, keepdims=True)
            s1 = i1[0, 0]
            s2 = i2[0, 0]
            idx_ref[0] = s1
            idx_ref[1] = s2
            b1 = pl.multiple_of((s1 // 16) * 16, 16)
            b2 = pl.multiple_of((s2 // 16) * 16, 16)
            row = lax.broadcasted_iota(jnp.int32, (16, D), 0)
            x1 = jnp.sum(jnp.where(row == s1 - b1, xn_ref[pl.ds(b1, 16), :].astype(f32), 0.0), axis=0, keepdims=True)
            x2 = jnp.sum(jnp.where(row == s2 - b2, xn_ref[pl.ds(b2, 16), :].astype(f32), 0.0), axis=0, keepdims=True)
            xs = jnp.where(row == 0, x1, jnp.where(row == 1, x2, 0.0)).astype(bf16)
            for c in w_copies():
                c.wait()
            g = jnp.dot(xs, wg_ref[...], preferred_element_type=f32)
            u = jnp.dot(xs, wu_ref[...], preferred_element_type=f32)
            hg = 0.5 * g
            hmid = ((hg + hg * jnp.tanh(hg)) * u).astype(bf16)
            y = jnp.dot(hmid, wd_ref[...], preferred_element_type=f32)
            rs = jnp.where(row[:8, :1] == 0, m1, m2)
            upd_ref[...] = y[0:8, :] * jax.nn.sigmoid(rs)

        c = (DH ** -0.5) * LOG2E

        @scope("main")
        def main(slot):
            z = jnp.zeros((64, W), bf16)
            k0p = jnp.concatenate([k_s[slot, 0], z], axis=0).T
            k1p = jnp.concatenate([z, k_s[slot, 1]], axis=0).T
            for i in range(nsub):
                sl = pl.ds(i * bm, bm)
                xn = xn_ref[sl, :]
                q = (jnp.dot(xn, wq_s[slot], preferred_element_type=f32) * c).astype(bf16)
                outs = []
                for (qq, kk, h) in ((q[:, 0:256], k0p, 0), (q[:, 128:384], k1p, 1)):
                    sT = lax.dot_general(kk, qq, NT, preferred_element_type=f32)
                    m = jnp.max(sT, axis=0, keepdims=True)
                    e = jnp.exp2(sT - m)
                    l = jnp.sum(e, axis=0, keepdims=True)
                    oT = jnp.dot(v_s[slot, h], e.astype(bf16), preferred_element_type=f32)
                    outs.append((oT * (1.0 / l)).astype(bf16))
                oT = jnp.concatenate(outs, axis=0)
                acc_ref[sl, :] += lax.dot_general(oT, wo_s[slot], TN, preferred_element_type=f32)

        def pair(p, carry):
            for cp in pair_copies(p):
                cp.wait()

            @pl.when(p + 1 < NP)
            def _():
                for cp in pair_copies(p + 1):
                    cp.start()

            @pl.when(p == rstep - 1)
            def _():
                for cp in w_copies():
                    cp.start()

            @pl.when(p == rstep)
            def _():
                router()

            main(p % 2)
            return carry

        if rstep == 0:
            for cp in w_copies():
                cp.start()
        lax.fori_loop(0, NP, pair, 0)

        @scope("fin")
        def fin_all():
            row = lax.broadcasted_iota(jnp.int32, (16, D), 0)
            for j in range(2):
                s = idx_ref[j]
                b = pl.multiple_of((s // 16) * 16, 16)
                blk = xn_ref[pl.ds(b, 16), :].astype(f32)
                xn_ref[pl.ds(b, 16), :] = (blk + jnp.where(row == s - b, upd_ref[j:j + 1, :], 0.0)).astype(bf16)

            def fin(i, carry):
                sl = pl.ds(pl.multiple_of(i * oc, oc), oc)
                hb = 0.5 * xn_ref[sl, :].astype(f32)
                g = hb + hb * jnp.tanh(hb)
                obuf[sl, :] = (xbuf[sl, :].astype(f32) + acc_ref[sl, :] * g).astype(bf16)
                o_copy(i).start()
                return carry
            lax.fori_loop(0, noc, fin, 0)
            for i in range(noc):
                o_copy(i).wait()
        fin_all()

    def fn(A_x, A_k_cache, A_v_cache, A_wq, A_wo, B_x, B_w_r, B_w_gate, B_w_up, B_w_down):
        x2 = A_x.reshape(S, D)
        kT = jnp.swapaxes(A_k_cache, 2, 3)
        vT = jnp.swapaxes(A_v_cache, 2, 3)
        anyspec = pl.BlockSpec(memory_space=pltpu.HBM)
        args = [x2, kT, vT, A_wq, A_wo, B_w_r.reshape(1, D), B_w_gate, B_w_up, B_w_down]
        args = [pltpu.with_memory_space_constraint(a, pltpu.HBM) for a in args]
        out = pl.pallas_call(
            kernel,
            in_specs=[
                anyspec, anyspec, anyspec, anyspec, anyspec,
                pl.BlockSpec((1, D), lambda: (0, 0)),
                anyspec, anyspec, anyspec,
            ],
            out_specs=anyspec,
            out_shape=jax.ShapeDtypeStruct((S, D), jnp.bfloat16),
            scratch_shapes=[
                pltpu.VMEM((S, D), bf16),
                pltpu.VMEM((S, D), bf16),
                pltpu.VMEM((S, D), f32),
                pltpu.VMEM((S, D), bf16),
                pltpu.VMEM((8, S), f32),
                pltpu.VMEM((D, F), bf16), pltpu.VMEM((D, F), bf16), pltpu.VMEM((F, D), bf16),
                pltpu.VMEM((8, D), f32),
                pltpu.SMEM((2,), jnp.int32),
                pltpu.VMEM((2, D, 2 * DH), bf16),
                pltpu.VMEM((2, 2, DH, W), bf16),
                pltpu.VMEM((2, 2, DH, W), bf16),
                pltpu.VMEM((2, 2 * DH, D), bf16),
                pltpu.SemaphoreType.DMA((nxc,)),
                pltpu.SemaphoreType.DMA((3,)),
                pltpu.SemaphoreType.DMA((noc,)),
                pltpu.SemaphoreType.DMA((4, 2)),
            ],
            compiler_params=pltpu.CompilerParams(vmem_limit_bytes=vmem * 1024 * 1024, flags=flags),
        )(*args)
        return out.reshape(1, S, D)
    return fn


_fn = make(bm=2048)


@jax.jit
def pallas_recurrent_scan__sliding_block_cached__moe_arch_mod__prompt_kernel(A_x, A_k_cache, A_v_cache, A_wq, A_wo, B_x, B_w_r, B_w_gate, B_w_up, B_w_down):
    return _fn(A_x, A_k_cache, A_v_cache, A_wq, A_wo, B_x, B_w_r, B_w_gate, B_w_up, B_w_down)
```

```python
import jax
import jax.numpy as jnp
from jax import lax
import jax.experimental.pallas as pl
import jax.experimental.pallas.tpu as pltpu

S, D, H, DH, SK, W, F = 2048, 640, 32, 192, 2048, 512, 1536
NP = H // 2
BM = 256
XC = 256
OC = 256
RSTEP = 2
LOG2E = 1.4426950408889634
NT = (((1,), (1,)), ((), ()))
TN = (((0,), (0,)), ((), ()))
f32 = jnp.float32
bf16 = jnp.bfloat16


def _kernel(x_hbm, k_hbm, v_hbm, wq_hbm, wo_hbm, wr_ref, wg_hbm, wu_hbm, wd_hbm, o_hbm,
            xbuf, xn_ref, acc_ref, obuf, r_ref, wg_ref, wu_ref, wd_ref, upd_ref, idx_ref,
            wq_s, k_s, v_s, wo_s, xsem, wsem, osem, qsem, ksem, vsem, psem):
    nsub, nxc, noc = S // BM, S // XC, S // OC

    def x_copy(i):
        r0 = pl.multiple_of(i * XC, XC)
        return pltpu.make_async_copy(x_hbm.at[pl.ds(r0, XC), :], xbuf.at[pl.ds(r0, XC), :], xsem.at[i])

    def o_copy(i):
        r0 = pl.multiple_of(i * OC, OC)
        return pltpu.make_async_copy(obuf.at[pl.ds(r0, OC), :], o_hbm.at[pl.ds(r0, OC), :], osem.at[i])

    def w_copies():
        return [pltpu.make_async_copy(wg_hbm, wg_ref, wsem.at[0]),
                pltpu.make_async_copy(wu_hbm, wu_ref, wsem.at[1]),
                pltpu.make_async_copy(wd_hbm, wd_ref, wsem.at[2])]

    def pair_copies(p):
        slot = p % 2
        c0 = pl.multiple_of(p * 2 * DH, 128)
        return [
            pltpu.make_async_copy(wq_hbm.at[:, pl.ds(c0, 2 * DH)], wq_s.at[slot], qsem.at[slot]),
            pltpu.make_async_copy(k_hbm.at[0, pl.ds(2 * p, 2), :, pl.ds(SK - W, W)], k_s.at[slot], ksem.at[slot]),
            pltpu.make_async_copy(v_hbm.at[0, pl.ds(2 * p, 2), :, pl.ds(SK - W, W)], v_s.at[slot], vsem.at[slot]),
            pltpu.make_async_copy(wo_hbm.at[pl.ds(c0, 2 * DH), :], wo_s.at[slot], psem.at[slot]),
        ]

    for i in range(nxc):
        x_copy(i).start()
    for cp in pair_copies(0):
        cp.start()

    wr8 = jnp.broadcast_to(wr_ref[...].astype(f32).reshape(1, D), (8, D)).astype(bf16)

    def layernorm(i, carry):
        x_copy(i).wait()
        sl = pl.ds(pl.multiple_of(i * XC, XC), XC)
        x = xbuf[sl, :].astype(f32)
        d = x - jnp.mean(x, axis=-1, keepdims=True)
        v = jnp.mean(d * d, axis=-1, keepdims=True)
        xn = (d * lax.rsqrt(v + 1e-5)).astype(bf16)
        xn_ref[sl, :] = xn
        r_ref[:, sl] = lax.dot_general(wr8, xn, NT, preferred_element_type=f32)
        acc_ref[sl, :] = jnp.zeros((XC, D), f32)
        return carry

    lax.fori_loop(0, nxc, layernorm, 0)

    def router():
        r = r_ref[...].astype(bf16).astype(f32)
        ii = lax.broadcasted_iota(jnp.int32, (8, S), 1)
        m1 = jnp.max(r, axis=1, keepdims=True)
        i1 = jnp.min(jnp.where(r == m1, ii, S - 1), axis=1, keepdims=True)
        r2 = jnp.where(ii == i1, -jnp.inf, r)
        m2 = jnp.max(r2, axis=1, keepdims=True)
        i2 = jnp.min(jnp.where((r2 == m2) & (ii != i1), ii, S - 1), axis=1, keepdims=True)
        s1 = i1[0, 0]
        s2 = i2[0, 0]
        idx_ref[0] = s1
        idx_ref[1] = s2
        b1 = pl.multiple_of((s1 // 16) * 16, 16)
        b2 = pl.multiple_of((s2 // 16) * 16, 16)
        row = lax.broadcasted_iota(jnp.int32, (16, D), 0)
        x1 = jnp.sum(jnp.where(row == s1 - b1, xn_ref[pl.ds(b1, 16), :].astype(f32), 0.0), axis=0, keepdims=True)
        x2 = jnp.sum(jnp.where(row == s2 - b2, xn_ref[pl.ds(b2, 16), :].astype(f32), 0.0), axis=0, keepdims=True)
        xs = jnp.where(row == 0, x1, jnp.where(row == 1, x2, 0.0)).astype(bf16)
        for c_ in w_copies():
            c_.wait()
        g = jnp.dot(xs, wg_ref[...], preferred_element_type=f32)
        u = jnp.dot(xs, wu_ref[...], preferred_element_type=f32)
        hg = 0.5 * g
        hmid = ((hg + hg * jnp.tanh(hg)) * u).astype(bf16)
        y = jnp.dot(hmid, wd_ref[...], preferred_element_type=f32)
        rs = jnp.where(row[:8, :1] == 0, m1, m2)
        upd_ref[...] = y[0:8, :] * jax.nn.sigmoid(rs)

    scale = (DH ** -0.5) * LOG2E

    def softmax(sT):
        m = jnp.max(sT, axis=0, keepdims=True)
        e = jnp.exp2(sT - m)
        l = jnp.sum(e, axis=0, keepdims=True)
        return e.astype(bf16), 1.0 / l

    def attention(slot):
        z = jnp.zeros((64, W), bf16)
        kp = [jnp.concatenate([k_s[slot, 0], z], axis=0).T,
              jnp.concatenate([z, k_s[slot, 1]], axis=0).T]
        qs = [(jnp.dot(xn_ref[pl.ds(i * BM, BM), :], wq_s[slot], preferred_element_type=f32) * scale).astype(bf16)
              for i in range(nsub)]
        ss = [[lax.dot_general(kp[h], q[:, 128 * h:128 * h + 256], NT, preferred_element_type=f32)
               for h in range(2)] for q in qs]
        ee = [[softmax(sT) for sT in s2] for s2 in ss]
        oo = [[(jnp.dot(v_s[slot, h], e2[h][0], preferred_element_type=f32) * e2[h][1]).astype(bf16)
               for h in range(2)] for e2 in ee]
        for i in range(nsub):
            oT = jnp.concatenate(oo[i], axis=0)
            acc_ref[pl.ds(i * BM, BM), :] += lax.dot_general(oT, wo_s[slot], TN, preferred_element_type=f32)

    def pair(p, carry):
        for cp in pair_copies(p):
            cp.wait()

        @pl.when(p + 1 < NP)
        def _():
            for cp in pair_copies(p + 1):
                cp.start()

        @pl.when(p == RSTEP - 1)
        def _():
            for cp in w_copies():
                cp.start()

        @pl.when(p == RSTEP)
        def _():
            router()

        attention(p % 2)
        return carry

    lax.fori_loop(0, NP, pair, 0)

    row = lax.broadcasted_iota(jnp.int32, (16, D), 0)
    for j in range(2):
        s = idx_ref[j]
        b = pl.multiple_of((s // 16) * 16, 16)
        blk = xn_ref[pl.ds(b, 16), :].astype(f32)
        xn_ref[pl.ds(b, 16), :] = (blk + jnp.where(row == s - b, upd_ref[j:j + 1, :], 0.0)).astype(bf16)

    def finish(i, carry):
        sl = pl.ds(pl.multiple_of(i * OC, OC), OC)
        hb = 0.5 * xn_ref[sl, :].astype(f32)
        g = hb + hb * jnp.tanh(hb)
        obuf[sl, :] = (xbuf[sl, :].astype(f32) + acc_ref[sl, :] * g).astype(bf16)
        o_copy(i).start()
        return carry

    lax.fori_loop(0, noc, finish, 0)
    for i in range(noc):
        o_copy(i).wait()


@jax.jit
def pallas_recurrent_scan__sliding_block_cached__moe_arch_mod__prompt_kernel(
        A_x, A_k_cache, A_v_cache, A_wq, A_wo, B_x, B_w_r, B_w_gate, B_w_up, B_w_down):
    hbm = pl.BlockSpec(memory_space=pltpu.HBM)
    out = pl.pallas_call(
        _kernel,
        in_specs=[hbm, hbm, hbm, hbm, hbm, pl.BlockSpec((D,), lambda: (0,)), hbm, hbm, hbm],
        out_specs=hbm,
        out_shape=jax.ShapeDtypeStruct((S, D), bf16),
        scratch_shapes=[
            pltpu.VMEM((S, D), bf16),
            pltpu.VMEM((S, D), bf16),
            pltpu.VMEM((S, D), f32),
            pltpu.VMEM((S, D), bf16),
            pltpu.VMEM((8, S), f32),
            pltpu.VMEM((D, F), bf16), pltpu.VMEM((D, F), bf16), pltpu.VMEM((F, D), bf16),
            pltpu.VMEM((8, D), f32),
            pltpu.SMEM((2,), jnp.int32),
            pltpu.VMEM((2, D, 2 * DH), bf16),
            pltpu.VMEM((2, 2, DH, W), bf16),
            pltpu.VMEM((2, 2, DH, W), bf16),
            pltpu.VMEM((2, 2 * DH, D), bf16),
            pltpu.SemaphoreType.DMA((S // XC,)),
            pltpu.SemaphoreType.DMA((3,)),
            pltpu.SemaphoreType.DMA((S // OC,)),
            pltpu.SemaphoreType.DMA((2,)),
            pltpu.SemaphoreType.DMA((2,)),
            pltpu.SemaphoreType.DMA((2,)),
            pltpu.SemaphoreType.DMA((2,)),
        ],
        compiler_params=pltpu.CompilerParams(vmem_limit_bytes=100 * 1024 * 1024),
    )(A_x.reshape(S, D), jnp.swapaxes(A_k_cache, 2, 3), jnp.swapaxes(A_v_cache, 2, 3),
      A_wq, A_wo, B_w_r, B_w_gate, B_w_up, B_w_down)
    return out.reshape(1, S, D)
```
